```python
import jax
import jax.numpy as jnp

def _softmax(x, axis=-1):
    return jax.nn.softmax(x, axis=axis)

def _gelu(x):
    return jax.nn.gelu(x, approximate=True)

def _silu(x):
    return jax.nn.silu(x)

def _sigmoid(x):
    return jax.nn.sigmoid(x)

def _layernorm(x, axis=-1, eps=1e-05):
    m = jnp.mean(x, axis=axis, keepdims=True)
    v = jnp.var(x, axis=axis, keepdims=True)
    return (x - m) / jnp.sqrt(v + eps)

def _scatter_add(tgt, idx, src, axis=0):
    return tgt.at[idx].add(src)

def _segment_sum(src, seg, n):
    return jax.ops.segment_sum(src, seg, n)

class _Rng:

    def __init__(self, key):
        self._k = key

    def _next(self):
        self._k, sub = jax.random.split(self._k)
        return sub

    def normal(self, shape):
        return jax.random.normal(self._next(), shape, dtype=jnp.bfloat16)

    def randint(self, lo, hi, shape):
        return jax.random.randint(self._next(), shape, lo, hi, dtype=jnp.int32)

    def uniform(self, shape, lo=0.0, hi=1.0):
        return jax.random.uniform(self._next(), shape, jnp.bfloat16, lo, hi)

    def permutation(self, n):
        return jax.random.permutation(self._next(), n)
kernel_name = 'interleave_layers__sliding_local_dilated__mixer_gmlp__prompt'

def setup_inputs():
    _rng = _Rng(jax.random.key(int.from_bytes(__import__("os").urandom(4), "little")))
    _w = lambda a: (lambda t: t.astype(jnp.bfloat16) if jnp.issubdtype(t.dtype, jnp.floating) else t)(jnp.asarray(a))

    def _A_setup():
        B, S, D = (1, 2048, 576)
        return {'x': _w((lambda *s: _rng.normal(s) * 0.05)(B, S, D)), 'wqkv': _w((lambda *s: _rng.normal(s) * 0.05)(D, 3 * D)), 'wo': _w((lambda *s: _rng.normal(s) * 0.05)(D, D))}
    _A_in = _A_setup()

    def _B_setup():
        B, S, D, F = (1, 2048, 576, 4608)
        Fh = F // 2
        return {'x': _w((lambda *s: _rng.normal(s) * 0.05)(B, S, D)), 'w_in': _w((lambda *s: _rng.normal(s) * 0.05)(D, 2 * Fh)), 'w_sp': _w(0.01 * (lambda *s: _rng.normal(s) * 0.05)(S, S)), 'b_sp': _w(1.0 + 0.01 * (lambda *s: _rng.normal(s) * 0.05)(S)), 'w_out': _w((lambda *s: _rng.normal(s) * 0.05)(Fh, D))}
    _B_in = _B_setup()
    return {'A_x': _A_in['x'], 'A_wqkv': _A_in['wqkv'], 'A_wo': _A_in['wo'], 'B_x': _B_in['x'], 'B_w_in': _B_in['w_in'], 'B_w_sp': _B_in['w_sp'], 'B_b_sp': _B_in['b_sp'], 'B_w_out': _B_in['w_out']}

def reference(A_x, A_wqkv, A_wo, B_x, B_w_in, B_w_sp, B_b_sp, B_w_out):

    def _A_ref(x, wqkv, wo):
        B, S, D = x.shape
        H = 32
        Dh = D // H
        W, dil = (8, 2)
        qkv = (lambda x, *d: x.transpose(*d))((x @ wqkv).reshape(B, S, 3, H, Dh), 2, 0, 3, 1, 4)
        q, k, v = (qkv[0], qkv[1], qkv[2])
        scale = Dh ** (-0.5)
        pos = jnp.arange(S)
        off = jnp.arange(W) * dil
        idx = pos[:, None] - off[None, :]
        mask = idx >= 0
        idx_c = jnp.where(mask, idx, 0).reshape(-1)
        kg = k[:, :, idx_c, :].reshape(B, H, S, W, Dh)
        vg = v[:, :, idx_c, :].reshape(B, H, S, W, Dh)
        logits = jnp.einsum('bhsd,bhswd->bhsw', q, kg) * scale
        logits = jnp.where(mask[None, None, :, :], logits, -1000000000.0)
        attn = _softmax(logits, axis=-1)
        o = jnp.einsum('bhsw,bhswd->bhsd', attn, vg)
        return (lambda x, *d: x.transpose(*d))(o, 0, 2, 1, 3).reshape(B, S, D) @ wo

    def _B_ref(x, w_in, w_sp, b_sp, w_out):
        B, S, D = x.shape
        F = w_in.shape[-1]
        Fh = F // 2
        z = _gelu(jnp.einsum('bsd,df->bsf', x, w_in))
        z1 = z[..., :Fh].copy()
        z2 = _layernorm(z[..., Fh:], axis=-1)
        g = jnp.einsum('ts,bsf->btf', w_sp, z2) + b_sp[None, :, None]
        return jnp.einsum('bsf,fd->bsd', z1 * g, w_out)
    x = A_x
    x = x + _A_ref(_layernorm(x, axis=-1), A_wqkv, A_wo)
    x = x + _B_ref(_layernorm(x, axis=-1), B_w_in, B_w_sp, B_b_sp, B_w_out)
    x = x + _A_ref(_layernorm(x, axis=-1), A_wqkv, A_wo)
    x = x + _B_ref(_layernorm(x, axis=-1), B_w_in, B_w_sp, B_b_sp, B_w_out)
    return x
```

```python
import functools

import jax
import jax.numpy as jnp
import numpy as np
from jax import lax
import jax.experimental.pallas as pl
import jax.experimental.pallas.tpu as pltpu

S = 2048
D = 576
H = 32
DH = 18
W = 8
DIL = 2
F = 4608
FH = F // 2
HALO = 16
EPS = 1e-5
M = 256
NC = S // M

f32 = jnp.float32
bf16 = jnp.bfloat16


def _dot(a, b):
    return lax.dot_general(a, b, (((1,), (0,)), ((), ())), preferred_element_type=f32)


def _ln(x):
    n = x.shape[-1]
    m = jnp.sum(x, axis=-1, keepdims=True) * (1.0 / n)
    c = x - m
    v = jnp.sum(c * c, axis=-1, keepdims=True) * (1.0 / n)
    return c * lax.rsqrt(v + EPS)


def _gelu(x):
    c1 = float(np.sqrt(2.0 / np.pi))
    c2 = c1 * 0.044715
    t = x * (c1 + c2 * (x * x))
    hx = 0.5 * x
    return hx * jnp.tanh(t) + hx


def _kernel(x_hbm, wqkv_hbm, wo_hbm, win_hbm, wsp_hbm, b_ref, wout_hbm, out_hbm,
            xin, xres, wqkv_raw, wo_raw, wp, wop, win, wsp, wout, bcol,
            kv, z1, z2a, z2b, zt, obuf, sems):
    cp_x = pltpu.make_async_copy(x_hbm, xin, sems.at[0])
    cp_qkv = pltpu.make_async_copy(wqkv_hbm, wqkv_raw, sems.at[1])
    cp_wo = pltpu.make_async_copy(wo_hbm, wo_raw, sems.at[2])
    cp_win = pltpu.make_async_copy(win_hbm, win, sems.at[3])
    cp_wsp = pltpu.make_async_copy(wsp_hbm, wsp, sems.at[4])
    cp_wout = pltpu.make_async_copy(wout_hbm, wout, sems.at[5])
    cp_qkv.start()
    cp_x.start()
    cp_wo.start()
    cp_win.start()
    cp_wsp.start()
    cp_wout.start()

    bb = b_ref[...].astype(f32)
    for r in range(S // 128):
        bcol[r * 128:(r + 1) * 128, :] = jnp.broadcast_to(bb[r:r + 1, :], (128, 128)).T

    rr = lax.broadcasted_iota(jnp.int32, (640, 640), 0)
    cc = lax.broadcasted_iota(jnp.int32, (640, 640), 1)
    src = (cc % H) * DH + cc // H
    p0 = jnp.where((rr == src) & (cc < D), 1.0, 0.0).astype(bf16)
    p64 = jnp.where((rr == src + 64) & (cc < D), 1.0, 0.0).astype(bf16)
    cp_qkv.wait()
    wq = _dot(wqkv_raw[:, 0:640], p0).astype(bf16)
    wk = _dot(wqkv_raw[:, 512:1152], p64).astype(bf16)
    wv = _dot(wqkv_raw[:, 1152:1728], p0[0:D, :]).astype(bf16)
    wp[:, 0:640] = wq
    wp[:, 640:1280] = wk
    wp[:, 1280:1920] = wv
    srcr = (rr % H) * DH + rr // H
    pt = jnp.where((cc == srcr) & (rr < D), 1.0, 0.0).astype(bf16)
    cp_wo.wait()
    wop[...] = _dot(pt[:, 0:D], wo_raw[...]).astype(bf16)

    scale = float(DH ** -0.5)

    def attn_part(c, x):
        xn = _ln(x).astype(bf16)
        qkv = _dot(xn, wp[...])
        q = qkv[:, 0:640] * scale
        kv[HALO:HALO + M, :] = qkv[:, 640:1920]
        row = c * M + lax.broadcasted_iota(jnp.int32, (M, 128), 0)
        lg = []
        for w in range(W):
            k = kv[HALO - DIL * w:HALO - DIL * w + M, 0:640]
            p = q * k
            s = p[:, 0:128] + p[:, 128:256] + p[:, 256:384] + p[:, 384:512] + p[:, 512:640]
            s = s + pltpu.roll(s, 64, 1)
            s = s + pltpu.roll(s, 32, 1)
            if w > 0:
                s = jnp.where(row >= DIL * w, s, -1e9)
            lg.append(s)
        mx = functools.reduce(jnp.maximum, lg)
        ex = [jnp.exp(l - mx) for l in lg]
        inv = 1.0 / functools.reduce(jnp.add, ex)
        o = None
        for w in range(W):
            a = ex[w] * inv
            v = kv[HALO - DIL * w:HALO - DIL * w + M, 640:1280]
            t = jnp.concatenate([a] * 5, axis=1) * v
            o = t if o is None else o + t
        kv[0:HALO, :] = kv[M:M + HALO, :]
        return x + _dot(o.astype(bf16), wop[...])

    def gmlp_in(c, x, z2dst):
        r0 = pl.multiple_of(c * M, M)
        xn = _ln(x).astype(bf16)
        z1[pl.ds(r0, M), :] = _gelu(_dot(xn, win[:, 0:FH])).astype(bf16)
        zt[...] = _gelu(_dot(xn, win[:, FH:F]))
        z2dst[pl.ds(r0, M), :] = _ln(zt[...]).astype(bf16)

    def gmlp_out(c, z2src):
        r0 = pl.multiple_of(c * M, M)
        g = _dot(wsp[pl.ds(r0, M), :], z2src[...])
        b = bcol[pl.ds(r0, M), :]
        g = g + jnp.concatenate([b] * (FH // 128), axis=1)
        h = (z1[pl.ds(r0, M), :].astype(f32) * g).astype(bf16)
        return xres[pl.ds(r0, M), :] + _dot(h, wout[...])

    kv[0:HALO, :] = jnp.zeros((HALO, 1280), f32)
    cp_x.wait()
    cp_win.wait()

    def ph1(c, _):
        r0 = pl.multiple_of(c * M, M)
        x = attn_part(c, xin[pl.ds(r0, M), :].astype(f32))
        xres[pl.ds(r0, M), :] = x
        gmlp_in(c, x, z2a)
        return 0

    lax.fori_loop(0, NC, ph1, 0)
    cp_wsp.wait()
    cp_wout.wait()

    def ph2(c, _):
        r0 = pl.multiple_of(c * M, M)
        x = gmlp_out(c, z2a)
        x = attn_part(c, x)
        xres[pl.ds(r0, M), :] = x
        gmlp_in(c, x, z2b)
        return 0

    kv[0:HALO, :] = jnp.zeros((HALO, 1280), f32)
    lax.fori_loop(0, NC, ph2, 0)

    def out_copy(c):
        r0 = pl.multiple_of(c * M, M)
        return pltpu.make_async_copy(xin.at[pl.ds(r0, M), :], out_hbm.at[pl.ds(r0, M), :], sems.at[6])

    def ph3(c, _):
        r0 = pl.multiple_of(c * M, M)
        xin[pl.ds(r0, M), :] = gmlp_out(c, z2b).astype(bf16)
        out_copy(c).start()
        return 0

    lax.fori_loop(0, NC, ph3, 0)
    pltpu.make_async_copy(xin, out_hbm, sems.at[6]).wait()


@jax.jit
def pallas_interleave_layers__sliding_local_dilated__mixer_gmlp__prompt_kernel(
    A_x: jax.Array,
    A_wqkv: jax.Array,
    A_wo: jax.Array,
    B_x: jax.Array,
    B_w_in: jax.Array,
    B_w_sp: jax.Array,
    B_b_sp: jax.Array,
    B_w_out: jax.Array,
):
    del B_x
    x = A_x.reshape(S, D)
    b = B_b_sp.reshape(S // 128, 128)
    any_spec = pl.BlockSpec(memory_space=pl.ANY)
    out = pl.pallas_call(
        _kernel,
        in_specs=[any_spec, any_spec, any_spec, any_spec, any_spec,
                  pl.BlockSpec(memory_space=pltpu.VMEM), any_spec],
        out_specs=any_spec,
        out_shape=jax.ShapeDtypeStruct((S, D), bf16),
        scratch_shapes=[
            pltpu.VMEM((S, D), bf16),
            pltpu.VMEM((S, D), f32),
            pltpu.VMEM((D, 3 * D), bf16),
            pltpu.VMEM((D, D), bf16),
            pltpu.VMEM((D, 1920), bf16),
            pltpu.VMEM((640, D), bf16),
            pltpu.VMEM((D, F), bf16),
            pltpu.VMEM((S, S), bf16),
            pltpu.VMEM((FH, D), bf16),
            pltpu.VMEM((S, 128), f32),
            pltpu.VMEM((HALO + M, 1280), f32),
            pltpu.VMEM((S, FH), bf16),
            pltpu.VMEM((S, FH), bf16),
            pltpu.VMEM((S, FH), bf16),
            pltpu.VMEM((M, FH), f32),
            pltpu.VMEM((M, D), bf16),
            pltpu.SemaphoreType.DMA((8,)),
        ],
        compiler_params=pltpu.CompilerParams(vmem_limit_bytes=110 * 1024 * 1024),
    )(x, A_wqkv, A_wo, B_w_in, B_w_sp, b, B_w_out)
    return out.reshape(1, S, D)
```

```python
import functools

import jax
import jax.numpy as jnp
import numpy as np
from jax import lax
import jax.experimental.pallas as pl
import jax.experimental.pallas.tpu as pltpu

S = 2048
D = 576
H = 32
DH = 18
W = 8
DIL = 2
F = 4608
FH = F // 2
EPS = 1e-5
N = 256
NC = S // N

f32 = jnp.float32
bf16 = jnp.bfloat16


def _dot(a, b):
    return lax.dot_general(a, b, (((1,), (0,)), ((), ())), preferred_element_type=f32)


def _dot_nt(a, b):
    return lax.dot_general(a, b, (((1,), (1,)), ((), ())), preferred_element_type=f32)


def _ln(x):
    n = x.shape[0]
    m = jnp.sum(x, axis=0, keepdims=True) * (1.0 / n)
    c = x - m
    v = jnp.sum(c * c, axis=0, keepdims=True) * (1.0 / n)
    return c * lax.rsqrt(v + EPS)


def _gelu(x):
    c1 = float(np.sqrt(2.0 / np.pi))
    c2 = c1 * 0.044715
    t = x * (c1 + c2 * (x * x))
    hx = 0.5 * x
    return hx * jnp.tanh(t) + hx


def _kernel(x_hbm, wqkv_hbm, wo_hbm, win_hbm, wsp_hbm, b_ref, wout_hbm, out_hbm,
            xin, xres, wqkv_raw, wo_raw, win_raw, wqkv, wo, win, wsp, wout,
            qb, kv, ob, z1, z2a, z2b, zt, xna, xnb, hb, sems):
    cp_x = pltpu.make_async_copy(x_hbm, xin, sems.at[0])
    cp_qkv = pltpu.make_async_copy(wqkv_hbm, wqkv_raw, sems.at[1])
    cp_wo = pltpu.make_async_copy(wo_hbm, wo_raw, sems.at[2])
    cp_win = pltpu.make_async_copy(win_hbm, win_raw, sems.at[3])
    cp_wsp = pltpu.make_async_copy(wsp_hbm, wsp, sems.at[4])
    cp_wout = pltpu.make_async_copy(wout_hbm, wout, sems.at[5])
    cp_qkv.start()
    cp_x.start()
    cp_wo.start()

    cp_qkv.wait()
    for j in range(0, 3 * D, 128):
        w = min(128, 3 * D - j)
        wqkv[j:j + w, :] = wqkv_raw[:, j:j + w].T

    scale = float(DH ** -0.5)
    NT = N // 128
    RB = 768

    def cols(c):
        return pl.ds(c * N, N) if isinstance(c, int) else pl.ds(pl.multiple_of(c * N, N), N)

    def run(*gens):
        st = [[g, 0.0, 1.0 / n] for g, n in gens]
        while st:
            e = min(st, key=lambda t: t[1])
            try:
                next(e[0])
                e[1] += e[2]
            except StopIteration:
                st.remove(e)

    def g_ln(load, store, rows, blk):
        acc = None
        for r in range(0, rows, blk):
            t = load(r, blk).reshape(blk // 8, 8, N).sum(axis=0)
            acc = t if acc is None else acc + t
            yield
        m = jnp.sum(acc, axis=0, keepdims=True) * (1.0 / rows)
        acc = None
        for r in range(0, rows, blk):
            t = load(r, blk) - m
            t = (t * t).reshape(blk // 8, 8, N).sum(axis=0)
            acc = t if acc is None else acc + t
            yield
        rs = lax.rsqrt(jnp.sum(acc, axis=0, keepdims=True) * (1.0 / rows) + EPS)
        for r in range(0, rows, blk):
            store(r, blk, ((load(r, blk) - m) * rs).astype(bf16))
            yield

    def g_lnx(c, dst):
        def store(r, n, v):
            dst[r:r + n, :] = v
        return g_ln(lambda r, n: xres[r:r + n, cols(c)], store, D, 64)

    def g_qkv():
        for r in range(0, 3 * D, 288):
            t = _dot(wqkv[r:r + 288, :], xna[...])
            for j in range(NT):
                if r < D:
                    qb[j, r:r + 288, :] = t[:, j * 128:(j + 1) * 128] * scale
                else:
                    kv[j + 1, (r - D) // 2:(r - D) // 2 + 144, :] = pltpu.bitcast(
                        t[:, j * 128:(j + 1) * 128].astype(bf16), jnp.uint32)
            yield

    def g_att(c):
        lane = lax.broadcasted_iota(jnp.int32, (H, 128), 1)

        def taps(j, r):
            k1 = kv[j + 1, pl.ds(r, H, stride=DH // 2), :]
            k0 = kv[j, pl.ds(r, H, stride=DH // 2), :]
            for w in range(W):
                sh = DIL * w
                u = k1 if w == 0 else pltpu.roll(jnp.where(lane >= 128 - sh, k0, k1), sh, 1)
                yield (lax.bitcast_convert_type(u << 16, f32),
                       lax.bitcast_convert_type(u & np.uint32(0xFFFF0000), f32))

        for j in range(NT):
            lg = [None] * W
            for d in range(DH // 2):
                qa = qb[j, pl.ds(2 * d, H, stride=DH), :]
                qc = qb[j, pl.ds(2 * d + 1, H, stride=DH), :]
                for w, (ka, kc) in enumerate(taps(j, d)):
                    p = qa * ka + qc * kc
                    lg[w] = p if d == 0 else lg[w] + p
                yield
            if j == 0:
                pos = c * N + lane
                lg = [l if w == 0 else jnp.where(pos >= DIL * w, l, -1e9) for w, l in enumerate(lg)]
            mx = functools.reduce(jnp.maximum, lg)
            ex = [jnp.exp(l - mx) for l in lg]
            inv = 1.0 / functools.reduce(jnp.add, ex)
            at = [e * inv for e in ex]
            for d in range(DH // 2):
                oa = oc = None
                for w, (va, vc) in enumerate(taps(j, D // 2 + d)):
                    ta = at[w] * va
                    tc = at[w] * vc
                    oa = ta if oa is None else oa + ta
                    oc = tc if oc is None else oc + tc
                ob[j, pl.ds(2 * d, H, stride=DH), :] = oa
                ob[j, pl.ds(2 * d + 1, H, stride=DH), :] = oc
                yield
        kv[0] = kv[NT]

    def g_wo(c):
        o = jnp.concatenate([ob[j] for j in range(NT)], axis=1).astype(bf16)
        for r in range(0, D, 288):
            xres[r:r + 288, cols(c)] += _dot(wo[r:r + 288, :], o)
            yield

    def g_in1(c):
        for r in range(0, FH, RB):
            z1[r:r + RB, cols(c)] = _gelu(_dot(win[r:r + RB, :], xnb[...])).astype(bf16)
            yield

    def g_in(c, dst):
        s1 = s2 = None
        for r in range(0, FH, RB):
            z = _gelu(_dot(win[FH + r:FH + r + RB, :], xnb[...]))
            zt[r:r + RB, :] = z
            t1 = z.reshape(RB // 32, 32, N).sum(axis=0)
            t2 = (z * z).reshape(RB // 32, 32, N).sum(axis=0)
            s1 = t1 if s1 is None else s1 + t1
            s2 = t2 if s2 is None else s2 + t2
            yield
        m = jnp.sum(s1, axis=0, keepdims=True) * (1.0 / FH)
        v = jnp.maximum(jnp.sum(s2, axis=0, keepdims=True) * (1.0 / FH) - m * m, 0.0)
        rs = lax.rsqrt(v + EPS)
        for r, _ in zip(range(0, FH, RB), g_in1(c)):
            dst[r:r + RB, cols(c)] = ((zt[r:r + RB, :] - m) * rs).astype(bf16)
            yield

    SB = 768

    def g_sp(c, src):
        b = b_ref[:, cols(c)].astype(f32)
        for r in range(0, FH, SB):
            g = _dot_nt(src[r:r + SB, :], wsp[cols(c), :]) + b
            hb[r:r + SB, :] = (z1[r:r + SB, cols(c)].astype(f32) * g).astype(bf16)
            yield

    def g_out(c, final=False):
        for r in range(0, D, 288):
            t = xres[r:r + 288, cols(c)] + _dot(wout[r:r + 288, :], hb[...])
            if final:
                xin[r:r + 288, cols(c)] = t.astype(bf16)
            else:
                xres[r:r + 288, cols(c)] = t
            yield

    NA = DH * NT
    NI = 2 * FH // RB
    NS = FH // SB
    kv[0] = jnp.zeros((D, 128), jnp.uint32)
    cp_x.wait()
    cp_wo.wait()
    cp_win.start()
    wo[...] = wo_raw[...].T
    xres[...] = xin[...].astype(f32)
    run((g_lnx(0, xna), 1))
    run((g_qkv(), 1))
    run((g_att(0), NA), (g_lnx(1, xna), 27))
    run((g_wo(0), 1))
    cp_win.wait()
    cp_wsp.start()
    cp_wout.start()
    for j in range(0, F, 128):
        win[j:j + 128, :] = win_raw[:, j:j + 128].T
    run((g_lnx(0, xnb), 27), (g_qkv(), 6))

    def ph1(c, _):
        run((g_att(c), NA), (g_in(c - 1, z2a), NI), (g_lnx(c + 1, xna), 27))
        run((g_wo(c), 1))
        run((g_lnx(c, xnb), 27), (g_qkv(), 6))
        return 0

    lax.fori_loop(1, NC - 1, ph1, 0)
    run((g_att(NC - 1), NA), (g_in(NC - 2, z2a), NI))
    run((g_wo(NC - 1), 1))
    run((g_lnx(NC - 1, xnb), 1))
    run((g_in(NC - 1, z2a), 1))
    cp_wsp.wait()
    cp_wout.wait()
    kv[0] = jnp.zeros((D, 128), jnp.uint32)
    run((g_sp(0, z2a), 1))
    run((g_out(0), 1))
    run((g_lnx(0, xna), 1))
    run((g_qkv(), 1))

    def ph2(c, _):
        run((g_att(c), NA), (g_sp(c + 1, z2a), NS))
        run((g_out(c + 1), 1))

        @pl.when(c > 0)
        def _():
            run((g_in(c - 1, z2b), 1))

        run((g_lnx(c + 1, xna), 27), (g_wo(c), 2))
        run((g_lnx(c, xnb), 27), (g_qkv(), 6))
        return 0

    lax.fori_loop(0, NC - 1, ph2, 0)
    run((g_att(NC - 1), NA), (g_in(NC - 2, z2b), NI))
    run((g_wo(NC - 1), 1))
    run((g_lnx(NC - 1, xnb), 1))
    run((g_in(NC - 1, z2b), 1))

    def out_copy(c):
        r0 = pl.multiple_of(c * N, N)
        return pltpu.make_async_copy(xin.at[:, pl.ds(r0, N)], out_hbm.at[:, pl.ds(r0, N)], sems.at[6])

    def ph3(c, _):
        r0 = pl.multiple_of(c * N, N)
        run((g_sp(c, z2b), 1))
        run((g_out(c, True), 1))
        out_copy(c).start()
        return 0

    lax.fori_loop(0, NC, ph3, 0)
    pltpu.make_async_copy(xin, out_hbm, sems.at[6]).wait()


@jax.jit
def pallas_interleave_layers__sliding_local_dilated__mixer_gmlp__prompt_kernel(
    A_x: jax.Array,
    A_wqkv: jax.Array,
    A_wo: jax.Array,
    B_x: jax.Array,
    B_w_in: jax.Array,
    B_w_sp: jax.Array,
    B_b_sp: jax.Array,
    B_w_out: jax.Array,
):
    del B_x
    x = A_x.reshape(S, D).T
    b = B_b_sp.reshape(1, S)
    any_spec = pl.BlockSpec(memory_space=pltpu.HBM)
    out = pl.pallas_call(
        _kernel,
        in_specs=[any_spec, any_spec, any_spec, any_spec, any_spec,
                  pl.BlockSpec(memory_space=pltpu.VMEM), any_spec],
        out_specs=any_spec,
        out_shape=jax.ShapeDtypeStruct((D, S), bf16),
        scratch_shapes=[
            pltpu.VMEM((D, S), bf16),
            pltpu.VMEM((D, S), f32),
            pltpu.VMEM((D, 3 * D), bf16),
            pltpu.VMEM((D, D), bf16),
            pltpu.VMEM((D, F), bf16),
            pltpu.VMEM((3 * D, D), bf16),
            pltpu.VMEM((D, D), bf16),
            pltpu.VMEM((F, D), bf16),
            pltpu.VMEM((S, S), bf16),
            pltpu.VMEM((D, FH), bf16),
            pltpu.VMEM((N // 128, D, 128), f32),
            pltpu.VMEM((N // 128 + 1, D, 128), jnp.uint32),
            pltpu.VMEM((N // 128, D, 128), f32),
            pltpu.VMEM((FH, S), bf16),
            pltpu.VMEM((FH, S), bf16),
            pltpu.VMEM((FH, S), bf16),
            pltpu.VMEM((FH, N), f32),
            pltpu.VMEM((D, N), bf16),
            pltpu.VMEM((D, N), bf16),
            pltpu.VMEM((FH, N), bf16),
            pltpu.SemaphoreType.DMA((8,)),
        ],
        compiler_params=pltpu.CompilerParams(vmem_limit_bytes=110 * 1024 * 1024),
    )(x, A_wqkv, A_wo, B_w_in, B_w_sp, b, B_w_out.T)
    return out.T.reshape(1, S, D)
```
